```python
import os as _os
_os.environ.setdefault("JAX_PLATFORMS", "cpu")
import jax
import jax.numpy as jnp

def _softmax(x, axis=-1):
    return jax.nn.softmax(x, axis=axis)
def _gelu(x):
    return jax.nn.gelu(x, approximate=True)
def _silu(x):
    return jax.nn.silu(x)
def _sigmoid(x):
    return jax.nn.sigmoid(x)
def _layernorm(x, axis=-1, eps=1e-5):
    m = jnp.mean(x, axis=axis, keepdims=True)
    v = jnp.var(x, axis=axis, keepdims=True)
    return (x - m) / jnp.sqrt(v + eps)
def _scatter_add(tgt, idx, src, axis=0):
    return tgt.at[idx].add(src)
def _segment_sum(src, seg, n):
    return jax.ops.segment_sum(src, seg, n)
class _Rng:
    def __init__(self, key):
        self._k = key
    def _next(self):
        self._k, sub = jax.random.split(self._k)
        return sub
    def normal(self, shape):
        return jax.random.normal(self._next(), shape, dtype=jnp.bfloat16)
    def randint(self, lo, hi, shape):
        return jax.random.randint(self._next(), shape, lo, hi, dtype=jnp.int32)
    def uniform(self, shape, lo=0.0, hi=1.0):
        return jax.random.uniform(self._next(), shape, jnp.bfloat16, lo, hi)
    def permutation(self, n):
        return jax.random.permutation(self._next(), n)


kernel_name = 'concat_heads__mha_block__ssm_conv_s4__prompt'

def setup_inputs():
    _rng = _Rng(jax.random.key(int.from_bytes(__import__("os").urandom(4), "little")))
    _w = (lambda a: (lambda t: t.astype(jnp.bfloat16) if jnp.issubdtype(t.dtype, jnp.floating) else t)(jnp.asarray(a)))
    def _A_setup():
        B, S, D, H = 1, 2048, 448, 16
        return {
            "x": _w((lambda *s: _rng.normal(s) * 0.2)(B, S, D)),
            "wqkv": _w((lambda *s: _rng.normal(s) * 0.2)(D, 3 * D)),
            "wo": _w((lambda *s: _rng.normal(s) * 0.05)(D, D)),
        }
    _A_in = _A_setup()

    def _B_setup():
        B, L, D, N = 1, 2048, 448, 256
        A_re = -jnp.exp((lambda *s: _rng.normal(s) * 0.2)(D, N))
        A_im = jnp.pi * (lambda *s: _rng.normal(s) * 0.2)(D, N)
        B_re = (lambda *s: _rng.normal(s) * 0.2)(D, N)
        B_im = (lambda *s: _rng.normal(s) * 0.2)(D, N)
        C_re = (lambda *s: _rng.normal(s) * 0.2)(D, N)
        C_im = (lambda *s: _rng.normal(s) * 0.2)(D, N)
        log_dt = (lambda *s: _rng.normal(s) * 0.2)(D) * 0.5 - 4.0
        Dskip = (lambda *s: _rng.normal(s) * 0.05)(D)
        return {
            "u": _w((lambda *s: _rng.normal(s) * 0.05)(B, L, D)),
            "A_re": _w(A_re),
            "A_im": _w(A_im),
            "B_re": _w(B_re),
            "B_im": _w(B_im),
            "C_re": _w(C_re),
            "C_im": _w(C_im),
            "log_dt": _w(log_dt),
            "Dskip": _w(Dskip),
        }
    _B_in = _B_setup()

    return {
        "A_x": _A_in["x"],
        "A_wqkv": _A_in["wqkv"],
        "A_wo": _A_in["wo"],
        "B_u": _B_in["u"],
        "B_A_re": _B_in["A_re"],
        "B_A_im": _B_in["A_im"],
        "B_B_re": _B_in["B_re"],
        "B_B_im": _B_in["B_im"],
        "B_C_re": _B_in["C_re"],
        "B_C_im": _B_in["C_im"],
        "B_log_dt": _B_in["log_dt"],
        "B_Dskip": _B_in["Dskip"],
    }

def reference(A_x, A_wqkv, A_wo, B_u, B_A_re, B_A_im, B_B_re, B_B_im, B_C_re, B_C_im, B_log_dt, B_Dskip):
    def _A_ref(x, wqkv, wo):
        B, S, D = x.shape
        H = 16
        Dh = D // H
        qkv = (lambda x, *d: x.transpose(*d))((x @ wqkv).reshape(B, S, 3, H, Dh), 2, 0, 3, 1, 4)
        q, k, v = qkv[0], qkv[1], qkv[2]
        scores = jnp.einsum("bhqd,bhkd->bhqk", q, k) * (Dh ** -0.5)
        p = _softmax(scores, axis=-1)
        o = jnp.einsum("bhqk,bhkd->bhqd", p, v)
        return (lambda x, *d: x.transpose(*d))(o, 0, 2, 1, 3).reshape(B, S, D) @ wo

    def _B_ref(u, A_re, A_im, B_re, B_im, C_re, C_im, log_dt, Dskip):
        Bsz, L, D = u.shape
        dt = jnp.exp(log_dt)[:, None]
        A = A_re + 1j * A_im
        Bc = B_re + 1j * B_im
        Cc = C_re + 1j * C_im
        logdA = dt * A
        dB = dt * Bc
        l = (lambda x, dt: x.astype(dt))(jnp.arange(L), A_re.dtype)
        P = jnp.exp(logdA[:, :, None] * l[None, None, :])
        K = jnp.einsum("dn,dnl,dn->dl", Cc, P, dB).real
        L2 = 2 * L
        Kp = jnp.pad(K, ((0, 0), (0, L)))
        up = (lambda x, *d: x.transpose(*d))(u, 0, 2, 1)
        up = jnp.pad(up, ((0, 0), (0, 0), (0, L)))
        Kf = (lambda x, axes=(-2,-1): jnp.fft.rfft2(x.astype(jnp.float32), axes=axes))(Kp[:, None, :], axes=(-2, -1))
        Uf = (lambda x, axes=(-2,-1): jnp.fft.rfft2(x.astype(jnp.float32), axes=axes))(up[:, :, None, :], axes=(-2, -1))
        Yf = Uf * Kf[None, :, :, :]
        y = (lambda x, s, axes=(-2,-1): jnp.fft.irfft2(x, s=s, axes=axes).astype(jnp.bfloat16))(Yf, (1, L2), axes=(-2, -1))[:, :, 0, :L]
        y = (lambda x, *d: x.transpose(*d))(y, 0, 2, 1) + u * Dskip[None, None, :]
        return y

    a = _A_ref(A_x, A_wqkv, A_wo)
    b = _B_ref(B_u, B_A_re, B_A_im, B_B_re, B_B_im, B_C_re, B_C_im, B_log_dt, B_Dskip)
    return jnp.concatenate([a, b], axis=-1)
```

```python
import functools

import numpy as np
import jax
import jax.numpy as jnp
import jax.experimental.pallas as pl
import jax.experimental.pallas.tpu as pltpu

S = 2048
D = 448
H = 16
DH = 28
HP = 32
DP = 512
NS = 256
LOFF = 64

TQ = 256
NC = 32
BR = 64
PAD = BR + 8

F32 = jnp.float32
BF16 = jnp.bfloat16


def _bf16_round_int(n):
    if n < 256:
        return n
    e = n.bit_length() - 8
    step = 1 << e
    lo = (n // step) * step
    rem = n - lo
    half = step // 2
    if rem > half or (rem == half and ((lo // step) & 1)):
        return lo + step
    return lo


_RL = [_bf16_round_int(l) for l in range(S)]
_SEGS = ((0, 1, 16), (256, 2, 8), (512, 4, 8), (1024, 8, 8))
_LAGS = []
for _b, _s, _na in _SEGS:
    _LAGS += [_b + _s * i for i in range(16 * _na)]
_LAGS.append(2048)
_LIDX = {v: i for i, v in enumerate(_LAGS)}
NLAG = len(_LAGS)
assert sorted(set(_RL)) == _LAGS and NLAG == 641

_plain = {}
_win = []
_groups = {}
for _l in range(S):
    _groups.setdefault(_RL[_l], []).append(_l)
for _v, _js in _groups.items():
    _key = (_js[0] - _v, _js[-1] - _v)
    if _key == (-1, 1):
        _win.append((8 if _v % 8 == 0 else 9, _v - (_v % 8), _LIDX[_v]))
    elif _key == (-2, 2):
        _win.append((10, _v, _LIDX[_v]))
    elif _key == (-3, 3):
        _win.append((11, _v, _LIDX[_v]))
    elif _key == (-4, 4):
        _win.append((12, _v, _LIDX[_v]))
    else:
        for _j in _js:
            _plain[_j] = _LIDX[_v]
for _j, _k in _plain.items():
    _win.append((_j % 8, _j - (_j % 8), _k))


def _make_runs(items):
    runs = []
    by_src = {}
    for src, lag, k in items:
        by_src.setdefault(src, []).append((lag, k))
    for src, lst in sorted(by_src.items()):
        lst.sort()
        i = 0
        while i < len(lst):
            if i + 1 < len(lst):
                dl = lst[i + 1][0] - lst[i][0]
                dk = lst[i + 1][1] - lst[i][1]
            else:
                dl, dk = 8, 0
            j = i + 1
            while j < len(lst) and lst[j][0] - lst[j - 1][0] == dl and lst[j][1] - lst[j - 1][1] == dk:
                j += 1
            runs.append((src, lst[i][0], dl, lst[i][1], dk, j - i))
            i = j
    return runs


_RUNS = _make_runs(_win)
NSRC = 13


def _cmul(ar, ai, br, bi):
    return ar * br - ai * bi, ar * bi + ai * br


def _kernel(x_ref, wq_ref, wk_ref, wv_ref, wo_ref, u_ref, are_ref, aim_ref, bre_ref, bim_ref,
            cre_ref, cim_ref, ldt_ref, dsk_ref, o_ref,
            qt_s, k_s, vt_s, ot_s, zr_s, zi_s, kacc_s, src_s):
    def proj(i, c):
        r = pl.multiple_of(i * 256, 256)
        xb = x_ref[pl.ds(r, 256), :]
        k_s[pl.ds(r, 256), :] = jnp.dot(xb, wk_ref[...], preferred_element_type=F32).astype(BF16)
        nt = (((1,), (1,)), ((), ()))
        qt_s[:, pl.ds(r, 256)] = jax.lax.dot_general(
            wq_ref[...], xb, nt, preferred_element_type=F32).astype(BF16)
        vt_s[:, pl.ds(r, 256)] = jax.lax.dot_general(
            wv_ref[...], xb, nt, preferred_element_type=F32).astype(BF16)
        return c
    jax.lax.fori_loop(0, S // 256, proj, 0)

    scale = float(np.asarray(DH ** -0.5, dtype=jnp.bfloat16).astype(np.float32))
    row_head = jax.lax.broadcasted_iota(jnp.int32, (128, TQ), 0) // HP

    def attn(it, c):
        h = it // (S // TQ)
        qb = it % (S // TQ)
        g = h // 4
        j = h % 4
        q0 = pl.multiple_of(qb * TQ, TQ)
        g0 = pl.multiple_of(g * 128, 128)
        qt = qt_s[pl.ds(g0, 128), pl.ds(q0, TQ)]
        qt = jnp.where(row_head == j, qt, jnp.zeros_like(qt))
        kk = k_s[:, pl.ds(g0, 128)]
        st = jnp.dot(kk, qt, preferred_element_type=F32)
        st = st.astype(BF16).astype(F32) * scale
        m = jnp.max(st, axis=0, keepdims=True)
        p = jnp.exp(st - m)
        l = jnp.sum(p, axis=0, keepdims=True)
        h0 = pl.multiple_of(h * HP, HP)
        vt = vt_s[pl.ds(h0, HP), :]
        ot = jnp.dot(vt, p.astype(BF16), preferred_element_type=F32)
        ot_s[pl.ds(h0, HP), pl.ds(q0, TQ)] = (ot / l).astype(BF16)
        return c
    jax.lax.fori_loop(0, H * (S // TQ), attn, 0)

    def oproj(i, c):
        r0 = pl.multiple_of(i * 256, 256)
        a = jax.lax.dot_general(ot_s[:, pl.ds(r0, 256)], wo_ref[...], (((0,), (0,)), ((), ())),
                                preferred_element_type=F32)
        o_ref[pl.ds(r0, 256), 0:512] = a.astype(BF16)
        return c
    jax.lax.fori_loop(0, S // 256, oproj, 0)

    dt = jnp.exp(ldt_ref[...].astype(F32)).astype(BF16).astype(F32)

    def kgen(ci, c):
        n0 = pl.multiple_of(ci * NC, NC)
        sl = (pl.ds(n0, NC), slice(None))
        rho = dt * are_ref[sl].astype(F32)
        th = dt * aim_ref[sl].astype(F32)
        dbr = dt * bre_ref[sl].astype(F32)
        dbi = dt * bim_ref[sl].astype(F32)
        cbr, cbi = _cmul(cre_ref[sl].astype(F32), cim_ref[sl].astype(F32), dbr, dbi)

        def cexp(mult):
            mag = jnp.exp(rho * mult)
            ang = th * mult
            return mag * jnp.cos(ang), mag * jnp.sin(ang)

        z1 = cexp(1.0)
        zb = cexp(256.0)
        zstep = z1
        zbase = (jnp.ones_like(rho), jnp.zeros_like(rho))
        lag0 = 0
        for si, (base, step, na) in enumerate(_SEGS):
            if si == 1:
                zbase = zb
            if si >= 1:
                zstep = _cmul(*zstep, *zstep)
            if si >= 2:
                zbase = _cmul(*zbase, *zbase)
            cur = (jnp.ones_like(rho), jnp.zeros_like(rho))
            for b in range(16):
                zr_s[b] = cur[0]
                zi_s[b] = cur[1]
                cur = _cmul(*cur, *zstep)
            z16 = cur
            w = _cmul(cbr, cbi, *zbase)

            def abody(a, w, lag0=lag0, z16=z16):
                wr, wi = w

                def bbody(b, cc):
                    t = wr * zr_s[b] - wi * zi_s[b]
                    t = t.reshape(NC // 8, 8, DP).sum(axis=0)
                    idx = lag0 + a * 16 + b

                    @pl.when(ci == 0)
                    def _():
                        kacc_s[idx] = t

                    @pl.when(ci != 0)
                    def _():
                        kacc_s[idx] += t
                    return cc
                jax.lax.fori_loop(0, 16, bbody, 0)
                return _cmul(wr, wi, *z16)
            w = jax.lax.fori_loop(0, na, abody, w)
            lag0 += 16 * na
        t = w[0].reshape(NC // 8, 8, DP).sum(axis=0)

        @pl.when(ci == 0)
        def _():
            kacc_s[NLAG - 1] = t

        @pl.when(ci != 0)
        def _():
            kacc_s[NLAG - 1] += t
        return c
    jax.lax.fori_loop(0, NS // NC, kgen, 0)

    def kred(i, c):
        t = kacc_s[i]
        kacc_s[i] = jnp.broadcast_to(jnp.sum(t, axis=0, keepdims=True), (8, DP))
        return c
    jax.lax.fori_loop(0, NLAG, kred, 0)

    for r in range(8):
        src_s[r, pl.ds(0, PAD + 16), :] = jnp.zeros((PAD + 16, DP), F32)
        src_s[r, pl.ds(S + PAD - 16, 272), :] = jnp.zeros((272, DP), F32)

    for i in range(S // 256):
        r0 = i * 256
        ub = u_ref[pl.ds(r0, 256), :].astype(F32)
        for r in range(8):
            src_s[r, pl.ds(PAD + r + r0, 256), :] = ub

    def wsum(i, c):
        r0 = pl.multiple_of(i * 256, 256)

        def sh(k):
            if k >= 0:
                return src_s[k, pl.ds(r0, 256), :]
            return src_s[8 + k, pl.ds(r0 + 8, 256), :]
        s3 = sh(0) + sh(1) + sh(-1)
        s5 = s3 + sh(2) + sh(-2)
        s7 = s5 + sh(3) + sh(-3)
        s9 = s7 + sh(4) + sh(-4)
        s3b = sh(4) + sh(5) + sh(3)
        src_s[8, pl.ds(r0, 256), :] = s3
        src_s[9, pl.ds(r0, 256), :] = s3b
        src_s[10, pl.ds(r0, 256), :] = s5
        src_s[11, pl.ds(r0, 256), :] = s7
        src_s[12, pl.ds(r0, 256), :] = s9
        return c
    jax.lax.fori_loop(0, (S + 256) // 256, wsum, 0)

    dsk = dsk_ref[...].astype(F32)

    def conv(i, c):
        t0 = i * BR
        acc = jnp.zeros((BR, DP), F32)
        for (src, lag, dl, k0, dk, cnt) in _RUNS:
            nmax = jnp.clip((t0 + BR + 8 - lag + dl - 1) // dl, 0, cnt)

            def body(e, acc, src=src, lag=lag, dl=dl, k0=k0, dk=dk):
                start = pl.multiple_of(t0 + PAD - lag - dl * e, 8)
                kb = kacc_s[k0 + dk * e]
                s = src_s[src, pl.ds(start, BR), :].reshape(BR // 8, 8, DP)
                return acc + (s * kb[None]).reshape(BR, DP)
            acc = jax.lax.fori_loop(0, nmax, body, acc)
        r0 = pl.multiple_of(t0, BR)
        y = acc.astype(BF16).astype(F32) + (u_ref[pl.ds(r0, BR), :].astype(F32) * dsk).astype(BF16).astype(F32)
        lane = jax.lax.broadcasted_iota(jnp.int32, (BR, 128), 1)
        o_ref[pl.ds(r0, BR), 384:512] = jnp.where(
            lane < 64, o_ref[pl.ds(r0, BR), 384:512], y[:, 0:128].astype(BF16))
        o_ref[pl.ds(r0, BR), 512:896] = y[:, 128:512].astype(BF16)
        return c
    jax.lax.fori_loop(0, S // BR, conv, 0)


@jax.jit
def pallas_concat_heads__mha_block__ssm_conv_s4__prompt_kernel(
    A_x: jax.Array,
    A_wqkv: jax.Array,
    A_wo: jax.Array,
    B_u: jax.Array,
    B_A_re: jax.Array,
    B_A_im: jax.Array,
    B_B_re: jax.Array,
    B_B_im: jax.Array,
    B_C_re: jax.Array,
    B_C_im: jax.Array,
    B_log_dt: jax.Array,
    B_Dskip: jax.Array,
):
    x = A_x.reshape(S, D)
    w = jnp.pad(A_wqkv.reshape(D, 3, H, DH), ((0, 0), (0, 0), (0, 0), (0, HP - DH)))
    wq_t = w[:, 0].reshape(D, DP).T
    wk = w[:, 1].reshape(D, DP)
    wv_t = w[:, 2].reshape(D, DP).T
    wo = jnp.pad(A_wo.reshape(H, DH, D), ((0, 0), (0, HP - DH), (0, DP - D))).reshape(DP, DP)
    u = jnp.pad(B_u.reshape(S, D), ((0, 0), (LOFF, 0)))

    def prep(p):
        return jnp.pad(p.T, ((0, 0), (LOFF, 0)))
    ldt = jnp.pad(B_log_dt.reshape(1, D), ((0, 0), (LOFF, 0)))
    dsk = jnp.pad(B_Dskip.reshape(1, D), ((0, 0), (LOFF, 0)))

    out = pl.pallas_call(
        _kernel,
        out_shape=jax.ShapeDtypeStruct((S, 2 * D), BF16),
        scratch_shapes=[
            pltpu.VMEM((DP, S), BF16),
            pltpu.VMEM((S, DP), BF16),
            pltpu.VMEM((DP, S), BF16),
            pltpu.VMEM((DP, S), BF16),
            pltpu.VMEM((16, NC, DP), F32),
            pltpu.VMEM((16, NC, DP), F32),
            pltpu.VMEM((NLAG, 8, DP), F32),
            pltpu.VMEM((NSRC, S + PAD + 256, DP), F32),
        ],
        compiler_params=pltpu.CompilerParams(vmem_limit_bytes=120 * 1024 * 1024),
    )(x, wq_t, wk, wv_t, wo, u, prep(B_A_re), prep(B_A_im), prep(B_B_re), prep(B_B_im),
      prep(B_C_re), prep(B_C_im), ldt, dsk)
    return out.reshape(1, S, 2 * D)
```

```python
import numpy as np
import jax
import jax.numpy as jnp
import jax.experimental.pallas as pl
import jax.experimental.pallas.tpu as pltpu

S = 2048
D = 448
H = 16
DH = 28
HP = 32
DP = 512
NS = 256
LOFF = 64

TQ = 256
NQ = S // TQ
NIT = H * NQ // 2
NC = 16
NCH = NS // NC
BR = 64
PADR = 200
NT = 5
WID = 128 * NT

SPI = 5 * NCH * 2 // (5 * NIT // 4)
IT_A = 3 * NCH // SPI
IT_B = 2 * NCH // SPI
IT_C = NIT - IT_A - IT_B
DPB = -(-D // (IT_B + IT_C))
DPC = -(-(D - DPB * IT_B) // IT_C)
UPC = -(-252 // IT_C)

F32 = jnp.float32
BF16 = jnp.bfloat16
U32 = jnp.uint32


def _bf16_round_int(n):
    if n < 256:
        return n
    step = 1 << (n.bit_length() - 8)
    lo = (n // step) * step
    rem = n - lo
    half = step // 2
    if rem > half or (rem == half and ((lo // step) & 1)):
        return lo + step
    return lo


_RL = [_bf16_round_int(l) for l in range(S)]
_LAGS = list(range(256)) + [256 + 2 * i for i in range(128)] + \
    [512 + 4 * i for i in range(128)] + [1024 + 8 * i for i in range(128)] + [2048]
_LIDX = {v: i for i, v in enumerate(_LAGS)}
NLAG = len(_LAGS)
assert sorted(set(_RL)) == _LAGS and NLAG == 641

_units = []
for _i in range(S // BR):
    _t0 = _i * BR
    for _g in range(8):
        _lag = 512 + 64 * _g
        if _lag <= _t0 + BR + 4:
            _units.append((0, 1, PADR + _t0 - _lag, PADR + _t0 - _lag, 8, 384 + 16 * _g, _t0))
    for _g in range(8):
        _lag = 1024 + 128 * _g
        if _lag <= _t0 + BR + 4:
            _units.append((2, 3, PADR + _t0 - _lag, PADR + _t0 - _lag - 8, 16, 512 + 16 * _g, _t0))
assert len(_units) <= IT_C * UPC
while len(_units) < IT_C * UPC:
    _units.append((0, 1, 128, 128, 16, 384, 0))
_UNITS = np.asarray(_units, np.int32)
RB = 200
NSRC = 7


def _cmul(ar, ai, br, bi):
    return ar * br - ai * bi, ar * bi + ai * br


def _csq(a):
    return _cmul(a[0], a[1], a[0], a[1])


def _kernel(tab_ref, x_ref, wq_ref, wk_ref, wv_ref, wo_ref, u_ref, ut_ref, prm_ref, ldt_ref, dsk_ref, o_ref,
            qt_s, k_s, vt_s, ot_s, sta, stb, ma, mb, par_s, kacc_s, kac2_s, kd_s, kt_s,
            up_s, src_s, yt_s, y_s):
    def kacc_get(idx):
        r = idx * 8 if isinstance(idx, int) else pl.multiple_of(idx * 8, 8)
        return jnp.concatenate([kacc_s[lb, pl.ds(r, 8), :] for lb in range(4)], axis=1)

    def kacc_set(idx, v):
        r = idx * 8 if isinstance(idx, int) else pl.multiple_of(idx * 8, 8)
        for lb in range(4):
            kacc_s[lb, pl.ds(r, 8), :] = v[:, 128 * lb: 128 * (lb + 1)]

    qscale = float(np.asarray(DH ** -0.5, dtype=jnp.bfloat16).astype(np.float32)) * float(np.log2(np.e))
    vrow = jax.lax.broadcasted_iota(jnp.int32, (DP, 256), 0) % HP

    dt = jnp.exp(ldt_ref[...].astype(F32)).astype(BF16).astype(F32)
    kacc_s[:, pl.ds(640 * 8, 8), :] = jnp.zeros((4, 8, 128), F32)
    kac2_s[...] = jnp.zeros(kac2_s.shape, F32)
    y_s[...] = jnp.zeros(y_s.shape, F32)
    yt_s[pl.ds(0, LOFF)] = jnp.zeros((LOFF, 16, 128), F32)
    up_s[pl.ds(0, PADR), :] = jnp.zeros((PADR, DP), F32)
    up_s[pl.ds(PADR + S, 8), :] = jnp.zeros((8, DP), F32)
    for i in range(S // 256):
        up_s[pl.ds(PADR + i * 256, 256), :] = u_ref[pl.ds(i * 256, 256), :].astype(F32)
    for s in range(NSRC - 1):
        src_s[s, pl.ds(0, PADR - 8), :] = jnp.zeros((PADR - 8, DP), F32)

    def proj(i):
        r = pl.multiple_of(i * 256, 256)
        xb = x_ref[pl.ds(r, 256), :]
        kk = jnp.dot(xb, wk_ref[...], preferred_element_type=F32).astype(BF16)
        for g in range(4):
            k_s[g, pl.ds(r, 256), :] = kk[:, 128 * g: 128 * (g + 1)]
        nt = (((1,), (1,)), ((), ()))
        q = jax.lax.dot_general(wq_ref[...], xb, nt, preferred_element_type=F32)
        qt_s[:, pl.ds(r, 256)] = (q.astype(BF16).astype(F32) * qscale).astype(BF16)
        v = jax.lax.dot_general(wv_ref[...], xb, nt, preferred_element_type=F32)
        vt_s[:, pl.ds(r, 256)] = jnp.where(vrow == DH, 1.0, v).astype(BF16)

    def kpre(ci):
        n0 = pl.multiple_of(ci * NC, NC)
        prm = [prm_ref[j, pl.ds(n0, NC), :].astype(F32) for j in range(6)]
        rho = dt * prm[0]
        th = dt * prm[1]
        cb = _cmul(prm[4], prm[5], dt * prm[2], dt * prm[3])

        def cexp(mult):
            mag = jnp.exp(rho * mult)
            ang = th * mult
            return mag * jnp.cos(ang), mag * jnp.sin(ang)

        z1 = cexp(1.0)
        z256 = cexp(256.0)
        z2 = _csq(z1)
        z4 = _csq(z2)
        z8 = _csq(z4)
        z128 = _csq(_csq(_csq(_csq(z8))))
        z512 = _csq(z256)
        z1024 = _csq(z512)
        z2048 = _csq(z1024)
        for typ, (zs, zb) in enumerate(((z1, None), (z1, z128), (z2, z256), (z4, z512), (z8, z1024))):
            w0 = cb if zb is None else _cmul(*cb, *zb)
            s = typ * NCH + ci
            par_s[s, 0] = zs[0]
            par_s[s, 1] = zs[1]
            par_s[s, 2] = w0[0]
            par_s[s, 3] = w0[1]
        t = _cmul(*cb, *z2048)[0]
        kacc_set(NLAG - 1, kacc_get(NLAG - 1) + (t[0:8] + t[8:16]))

    def srcprep(i):
        a0 = pl.multiple_of(PADR - 8 + i * RB, 8)
        xw = up_s[pl.ds(a0 - 8, RB + 16), :]

        def sh(k):
            return xw[8 - k: 8 - k + RB]
        s3 = sh(0) + sh(1) + sh(-1)
        s5 = s3 + sh(2) + sh(-2)
        s7 = s5 + sh(3) + sh(-3)
        s9 = s7 + sh(4) + sh(-4)
        src_s[0, pl.ds(a0, RB), :] = s5
        src_s[1, pl.ds(a0, RB), :] = sh(3) + sh(4) + sh(5)
        src_s[2, pl.ds(a0, RB), :] = s9
        src_s[3, pl.ds(a0, RB), :] = s7
        src_s[4, pl.ds(a0, RB), :] = -sh(-2)
        src_s[5, pl.ds(a0, RB), :] = -(sh(-3) + sh(-4))

    def loop_p(i, c):
        proj(i)
        for q in range(NCH // 8):
            kpre(i * (NCH // 8) + q)
        srcprep(i)
        return c
    jax.lax.fori_loop(0, 8, loop_p, 0)
    xw = up_s[pl.ds(PADR - 128, 136), :]
    src_s[6, pl.ds(PADR - 128, 128), :] = xw[1:129] + xw[2:130] + xw[3:131] + xw[4:132]

    row_head = jax.lax.broadcasted_iota(jnp.int32, (128, TQ), 0) // HP

    def scores(it, st_ref, m_ref):
        h = it // NQ
        qb = it % NQ
        q0 = pl.multiple_of(qb * TQ, TQ)
        g0 = pl.multiple_of((h // 4) * 128, 128)
        qt = qt_s[pl.ds(g0, 128), pl.ds(q0, TQ)]
        qt = jnp.where(row_head == h % 4, qt, jnp.zeros_like(qt))
        st = jnp.dot(k_s[h // 4], qt, preferred_element_type=F32)
        st_ref[...] = st
        m_ref[...] = jnp.max(st, axis=0, keepdims=True)

    def finish(it, st_ref, m_ref):
        h = it // NQ
        qb = it % NQ
        q0 = pl.multiple_of(qb * TQ, TQ)
        p = jnp.exp2(st_ref[...] - m_ref[...]).astype(BF16)
        h0 = pl.multiple_of(h * HP, HP)
        ot = jnp.dot(vt_s[pl.ds(h0, HP), :], p, preferred_element_type=F32)
        ot_s[pl.ds(h0, HP), pl.ds(q0, TQ)] = (ot / ot[DH:DH + 1, :]).astype(BF16)

    def attn_pair(i):
        it = 2 * i
        scores(it + 1, stb, mb)
        finish(it, sta, ma)
        scores(jnp.minimum(it + 2, 2 * NIT - 1), sta, ma)
        finish(it + 1, stb, mb)

    def kslice(sl):
        typ = sl // NCH
        zs = (par_s[sl, 0], par_s[sl, 1])
        w = (par_s[sl, 2], par_s[sl, 3])
        z16 = _csq(_csq(_csq(_csq(zs))))
        c1 = zs[0] + zs[0]
        c2 = zs[0] * zs[0] + zs[1] * zs[1]
        base = typ * 128
        for a in range(8):
            r0 = w[0]
            r1 = r0 * zs[0] - w[1] * zs[1]
            for b in range(16):
                if b >= 2:
                    r0, r1 = r1, c1 * r1 - c2 * r0
                t = r0 if b == 0 else r1
                r = pl.multiple_of((base + a * 16 + b) * 8, 8)
                kac2_s[pl.ds(r, 8), :] += t[0:8] + t[8:16]
            if a < 7:
                w = _cmul(*w, *z16)

    def kslices(s0, n):
        for q in range(n):
            kslice(s0 + q)

    def kcopy(lo, hi):
        def body(j, c):
            r = pl.multiple_of((lo + 8 * j) * 8, 64)
            v = kac2_s[pl.ds(r, 64), :]
            for lb in range(4):
                kacc_s[lb, pl.ds(r, 64), :] = v[:, 128 * lb: 128 * (lb + 1)]
            return c
        jax.lax.fori_loop(0, (hi - lo) // 8, body, 0)

    def conv_d(d):
        r0 = kt_s[pl.ds(d, 1), :].astype(BF16).astype(F32)
        b0 = jax.lax.bitcast_convert_type(r0, U32)
        b1 = jax.lax.bitcast_convert_type(pltpu.roll(r0, 1, 1), U32)
        word = (b0 >> 16) | b1
        t32 = pltpu.roll(jnp.broadcast_to(word, (64, WID)), 0, 1, stride=2, stride_axis=0)
        w = pltpu.bitcast(t32, BF16)
        up = jnp.concatenate([jnp.zeros((16, 128), F32), ut_ref[d].astype(F32)], axis=0)
        acc = None
        for m in range(NT):
            t = jnp.dot(up[16 - m: 32 - m].astype(BF16), w[:, 128 * m: 128 * (m + 1)],
                        preferred_element_type=F32)
            acc = t if acc is None else acc + t
        yt_s[d] = acc

    def unit(ui):
        sa = tab_ref[ui, 0]
        sb = tab_ref[ui, 1]
        ra = tab_ref[ui, 2]
        rb = tab_ref[ui, 3]
        da = tab_ref[ui, 4]
        k0 = tab_ref[ui, 5]
        t0 = pl.multiple_of(tab_ref[ui, 6], BR)
        acc = y_s[pl.ds(t0, BR), :].reshape(BR // 8, 8, DP)
        for e in range(8):
            a = src_s[sa, pl.ds(pl.multiple_of(ra - da * e, 8), BR), :].reshape(BR // 8, 8, DP)
            b = src_s[sb, pl.ds(pl.multiple_of(rb - da * e, 8), BR), :].reshape(BR // 8, 8, DP)
            acc = acc + a * kacc_get(k0 + 2 * e)[None] + b * kacc_get(k0 + 2 * e + 1)[None]
        y_s[pl.ds(t0, BR), :] = acc.reshape(BR, DP)

    def kreduce(lo, hi):
        def body(j, c):
            r = pl.multiple_of((lo + 8 * j) * 8, 64)
            for lb in range(4):
                t = kacc_s[lb, pl.ds(r, 8, stride=8), :]
                for s in range(1, 8):
                    t = t + kacc_s[lb, pl.ds(r + s, 8, stride=8), :]
                kd_s[pl.ds(pl.multiple_of(lo + 8 * j, 8), 8), pl.ds(128 * lb, 128)] = t
            return c
        jax.lax.fori_loop(0, (hi - lo) // 8, body, 0)

    scores(0, sta, ma)

    def loop_a(i, c):
        attn_pair(i)
        kslices(SPI * i, SPI)
        return c
    jax.lax.fori_loop(0, IT_A, loop_a, 0)

    kcopy(0, 384)
    kreduce(0, 384)
    sub = jax.lax.broadcasted_iota(jnp.int32, (8, DP), 0)
    for blk in range(4):
        if blk < 2:
            rows = kd_s[pl.ds(128 * blk, 128), :]
        else:
            parts = []
            for b8 in range(16):
                acc = None
                for r in range(8):
                    l = 128 * blk + 8 * b8 + r
                    if l == 511:
                        v = jnp.zeros((8, DP), F32)
                    else:
                        v = jnp.broadcast_to(kd_s[pl.ds(_LIDX[_RL[l]], 1), :], (8, DP))
                    acc = v if acc is None else jnp.where(sub == r, v, acc)
                parts.append(acc)
            rows = jnp.concatenate(parts, axis=0)
        kt_s[:, pl.ds(128 * blk, 128)] = rows.T
    kt_s[:, pl.ds(512, 128)] = jnp.zeros((DP, 128), F32)

    def loop_b(j, c):
        attn_pair(IT_A + j)
        kslices(SPI * (IT_A + j), SPI)
        for q in range(DPB):
            conv_d(LOFF + j * DPB + q)
        return c
    jax.lax.fori_loop(0, IT_B, loop_b, 0)

    kcopy(384, 640)
    kreduce(384, 640)
    t = kacc_get(NLAG - 1)
    kd_s[pl.ds(640, 8), :] = jnp.broadcast_to(jnp.sum(t, axis=0, keepdims=True), (8, DP))

    def kbro(i, c):
        kacc_set(384 + i, jnp.broadcast_to(kd_s[pl.ds(384 + i, 1), :], (8, DP)))
        return c
    jax.lax.fori_loop(0, 257, kbro, 0)

    def loop_c(j, c):
        attn_pair(IT_A + IT_B + j)
        for q in range(UPC):
            unit(j * UPC + q)
        for q in range(DPC):
            conv_d(jnp.minimum(LOFF + IT_B * DPB + j * DPC + q, DP - 1))
        return c
    jax.lax.fori_loop(0, IT_C, loop_c, 0)

    dsk = dsk_ref[...].astype(F32)
    lane = jax.lax.broadcasted_iota(jnp.int32, (128, 128), 1)
    k512 = kacc_get(384)[None]
    k1024 = kacc_get(512)[None]
    k2048 = kacc_get(640)[None]

    def fin(tb, c):
        r0 = pl.multiple_of(tb * 128, 128)
        y = y_s[pl.ds(r0, 128), :]
        for s, lag, kk in ((4, 512, k512), (5, 1024, k1024), (6, 2048, k2048)):
            a = jnp.maximum(PADR + r0 - lag, PADR - 128)
            e = src_s[s, pl.ds(pl.multiple_of(a, 8), 128), :]
            valid = (PADR + r0 - lag) >= PADR - 128
            e = jnp.where(valid, e, 0.0)
            y = y + (e.reshape(16, 8, DP) * kk).reshape(128, DP)
        yt = jnp.concatenate([yt_s[pl.ds(128 * db, 128), tb, :].T for db in range(4)], axis=1)
        y = y + yt
        ud = (u_ref[pl.ds(r0, 128), :].astype(F32) * dsk).astype(BF16).astype(F32)
        y = (y.astype(BF16).astype(F32) + ud).astype(BF16)
        a = jax.lax.dot_general(ot_s[:, pl.ds(r0, 128)], wo_ref[...], (((0,), (0,)), ((), ())),
                                preferred_element_type=F32).astype(BF16)
        o_ref[pl.ds(r0, 128), 0:384] = a[:, 0:384]
        o_ref[pl.ds(r0, 128), 384:512] = jnp.where(lane < LOFF, a[:, 384:512], y[:, 0:128])
        o_ref[pl.ds(r0, 128), 512:896] = y[:, 128:512]
        return c
    jax.lax.fori_loop(0, S // 128, fin, 0)


@jax.jit
def pallas_concat_heads__mha_block__ssm_conv_s4__prompt_kernel(
    A_x: jax.Array,
    A_wqkv: jax.Array,
    A_wo: jax.Array,
    B_u: jax.Array,
    B_A_re: jax.Array,
    B_A_im: jax.Array,
    B_B_re: jax.Array,
    B_B_im: jax.Array,
    B_C_re: jax.Array,
    B_C_im: jax.Array,
    B_log_dt: jax.Array,
    B_Dskip: jax.Array,
):
    x = A_x.reshape(S, D)
    w = jnp.pad(A_wqkv.reshape(D, 3, H, DH), ((0, 0), (0, 0), (0, 0), (0, HP - DH)))
    wq_t = w[:, 0].reshape(D, DP).T
    wk = w[:, 1].reshape(D, DP)
    wv_t = w[:, 2].reshape(D, DP).T
    wo = jnp.pad(A_wo.reshape(H, DH, D), ((0, 0), (0, HP - DH), (0, DP - D))).reshape(DP, DP)
    u = jnp.pad(B_u.reshape(S, D), ((0, 0), (LOFF, 0)))
    ut = u.T.reshape(DP, 16, 128)

    prm = jnp.stack([B_A_re, B_A_im, B_B_re, B_B_im, B_C_re, B_C_im])
    prm = jnp.pad(prm.transpose(0, 2, 1), ((0, 0), (0, 0), (LOFF, 0)))
    ldt = jnp.pad(B_log_dt.reshape(1, D), ((0, 0), (LOFF, 0)))
    dsk = jnp.pad(B_Dskip.reshape(1, D), ((0, 0), (LOFF, 0)))

    vmem = pl.BlockSpec(memory_space=pltpu.VMEM)
    out = pl.pallas_call(
        _kernel,
        out_shape=jax.ShapeDtypeStruct((S, 2 * D), BF16),
        in_specs=[pl.BlockSpec(memory_space=pltpu.SMEM)] + [vmem] * 10,
        out_specs=vmem,
        scratch_shapes=[
            pltpu.VMEM((DP, S), BF16),
            pltpu.VMEM((4, S, 128), BF16),
            pltpu.VMEM((DP, S), BF16),
            pltpu.VMEM((DP, S), BF16),
            pltpu.VMEM((S, TQ), F32),
            pltpu.VMEM((S, TQ), F32),
            pltpu.VMEM((1, TQ), F32),
            pltpu.VMEM((1, TQ), F32),
            pltpu.VMEM((5 * NCH, 4, NC, DP), F32),
            pltpu.VMEM((4, (NLAG + 7) * 8, 128), F32),
            pltpu.VMEM((640 * 8, DP), F32),
            pltpu.VMEM((NLAG + 7, DP), F32),
            pltpu.VMEM((DP, WID), F32),
            pltpu.VMEM((S + PADR + 8, DP), F32),
            pltpu.VMEM((NSRC, S + PADR, DP), F32),
            pltpu.VMEM((DP, 16, 128), F32),
            pltpu.VMEM((S, DP), F32),
        ],
        compiler_params=pltpu.CompilerParams(vmem_limit_bytes=120 * 1024 * 1024),
    )(jnp.asarray(_UNITS), x, wq_t, wk, wv_t, wo, u, ut, prm, ldt, dsk)
    return out.reshape(1, S, 2 * D)
```

```python
import numpy as np
import jax
import jax.numpy as jnp
import jax.experimental.pallas as pl
import jax.experimental.pallas.tpu as pltpu

S = 2048
D = 448
H = 16
DH = 28
HP = 32
DP = 512
NS = 256
LOFF = 64

TQ = 256
NQ = S // TQ
NIT = H * NQ // 2
NC = 16
NCH = NS // NC
BR = 64
PADR = 200
NT = 5
WID = 128 * NT

SPI = 5 * NCH * 2 // (5 * NIT // 4)
IT_A = 3 * NCH // SPI
IT_B = 2 * NCH // SPI
IT_C = NIT - IT_A - IT_B
DPB = -(-D // (IT_B + IT_C))
DPC = -(-(D - DPB * IT_B) // IT_C)

F32 = jnp.float32
BF16 = jnp.bfloat16
U32 = jnp.uint32


def _bf16_round_int(n):
    if n < 256:
        return n
    step = 1 << (n.bit_length() - 8)
    lo = (n // step) * step
    rem = n - lo
    half = step // 2
    if rem > half or (rem == half and ((lo // step) & 1)):
        return lo + step
    return lo


_RL = [_bf16_round_int(l) for l in range(S)]
_LAGS = list(range(256)) + [256 + 2 * i for i in range(128)] + \
    [512 + 4 * i for i in range(128)] + [1024 + 8 * i for i in range(128)] + [2048]
_LIDX = {v: i for i, v in enumerate(_LAGS)}
NLAG = len(_LAGS)
assert sorted(set(_RL)) == _LAGS and NLAG == 641

_u2, _u3 = [], []
for _i in range(S // BR):
    _t0 = _i * BR
    for _g in range(8):
        _lag = 512 + 64 * _g
        if _lag <= _t0 + BR + 4:
            _u2.append((PADR + _t0 - _lag, 384 + 16 * _g, _t0))
    for _g in range(8):
        _lag = 1024 + 128 * _g
        if _lag <= _t0 + BR + 4:
            _u3.append((PADR + _t0 - _lag, 512 + 16 * _g, _t0))
U2PC = -(-len(_u2) // IT_C)
U3PC = -(-len(_u3) // IT_C)
while len(_u2) < IT_C * U2PC:
    _u2.append((128, 384, 0))
while len(_u3) < IT_C * U3PC:
    _u3.append((128, 384, 0))
_UNITS = np.asarray(_u2 + _u3, np.int32)
NU2 = len(_u2)
RB = 200
NSRC = 7


def _cmul(ar, ai, br, bi):
    return ar * br - ai * bi, ar * bi + ai * br


def _csq(a):
    return _cmul(a[0], a[1], a[0], a[1])


def _kernel(tab_ref, x_ref, wq_ref, wk_ref, wv_ref, wo_ref, u_ref, ut_ref, prm_ref, ldt_ref, dsk_ref, o_ref,
            qt_s, k_s, vt_s, ot_s, sta, stb, ma, mb, par_s, kacc_s, kac2_s, kd_s, kt_s,
            up_s, src_s, yt_s, y_s):
    def kacc_get(idx):
        r = idx * 8 if isinstance(idx, int) else pl.multiple_of(idx * 8, 8)
        return jnp.concatenate([kacc_s[lb, pl.ds(r, 8), :] for lb in range(4)], axis=1)

    def kacc_set(idx, v):
        r = idx * 8 if isinstance(idx, int) else pl.multiple_of(idx * 8, 8)
        for lb in range(4):
            kacc_s[lb, pl.ds(r, 8), :] = v[:, 128 * lb: 128 * (lb + 1)]

    qscale = float(np.asarray(DH ** -0.5, dtype=jnp.bfloat16).astype(np.float32)) * float(np.log2(np.e))
    vrow = jax.lax.broadcasted_iota(jnp.int32, (DP, 256), 0) % HP

    dt = jnp.exp(ldt_ref[...].astype(F32)).astype(BF16).astype(F32)
    kacc_s[:, pl.ds(640 * 8, 8), :] = jnp.zeros((4, 8, 128), F32)
    kac2_s[...] = jnp.zeros(kac2_s.shape, F32)
    y_s[...] = jnp.zeros(y_s.shape, F32)
    yt_s[pl.ds(0, LOFF)] = jnp.zeros((LOFF, 16, 128), F32)
    up_s[pl.ds(0, PADR), :] = jnp.zeros((PADR, DP), F32)
    up_s[pl.ds(PADR + S, 8), :] = jnp.zeros((8, DP), F32)
    for i in range(S // 256):
        up_s[pl.ds(PADR + i * 256, 256), :] = u_ref[pl.ds(i * 256, 256), :].astype(F32)
    for s in range(NSRC - 1):
        src_s[s, pl.ds(0, PADR - 8), :] = jnp.zeros((PADR - 8, DP), F32)

    def proj(i):
        r = pl.multiple_of(i * 256, 256)
        xb = x_ref[pl.ds(r, 256), :]
        kk = jnp.dot(xb, wk_ref[...], preferred_element_type=F32).astype(BF16)
        for g in range(4):
            k_s[g, pl.ds(r, 256), :] = kk[:, 128 * g: 128 * (g + 1)]
        nt = (((1,), (1,)), ((), ()))
        q = jax.lax.dot_general(wq_ref[...], xb, nt, preferred_element_type=F32)
        qt_s[:, pl.ds(r, 256)] = (q.astype(BF16).astype(F32) * qscale).astype(BF16)
        v = jax.lax.dot_general(wv_ref[...], xb, nt, preferred_element_type=F32)
        vt_s[:, pl.ds(r, 256)] = jnp.where(vrow == DH, 1.0, v).astype(BF16)

    def kpre(ci):
        n0 = pl.multiple_of(ci * NC, NC)
        prm = [prm_ref[j, pl.ds(n0, NC), :].astype(F32) for j in range(6)]
        rho = dt * prm[0]
        th = dt * prm[1]
        cb = _cmul(prm[4], prm[5], dt * prm[2], dt * prm[3])

        def cexp(mult):
            mag = jnp.exp(rho * mult)
            ang = th * mult
            return mag * jnp.cos(ang), mag * jnp.sin(ang)

        z1 = cexp(1.0)
        z256 = cexp(256.0)
        z2 = _csq(z1)
        z4 = _csq(z2)
        z8 = _csq(z4)
        z128 = _csq(_csq(_csq(_csq(z8))))
        z512 = _csq(z256)
        z1024 = _csq(z512)
        z2048 = _csq(z1024)
        for typ, (zs, zb) in enumerate(((z1, None), (z1, z128), (z2, z256), (z4, z512), (z8, z1024))):
            w0 = cb if zb is None else _cmul(*cb, *zb)
            s = typ * NCH + ci
            par_s[s, 0] = zs[0]
            par_s[s, 1] = zs[1]
            par_s[s, 2] = w0[0]
            par_s[s, 3] = w0[1]
        t = _cmul(*cb, *z2048)[0]
        kacc_set(NLAG - 1, kacc_get(NLAG - 1) + (t[0:8] + t[8:16]))

    def srcprep(i):
        a0 = pl.multiple_of(PADR - 8 + i * RB, 8)
        xw = up_s[pl.ds(a0 - 8, RB + 16), :]

        def sh(k):
            return xw[8 - k: 8 - k + RB]
        s3 = sh(0) + sh(1) + sh(-1)
        s5 = s3 + sh(2) + sh(-2)
        s7 = s5 + sh(3) + sh(-3)
        s9 = s7 + sh(4) + sh(-4)
        src_s[0, pl.ds(a0, RB), :] = s5
        src_s[1, pl.ds(a0, RB), :] = sh(3) + sh(4) + sh(5)
        src_s[2, pl.ds(a0, RB), :] = s9
        src_s[3, pl.ds(a0, RB), :] = s7
        src_s[4, pl.ds(a0, RB), :] = -sh(-2)
        src_s[5, pl.ds(a0, RB), :] = -(sh(-3) + sh(-4))

    def loop_p(i, c):
        proj(i)
        for q in range(NCH // 8):
            kpre(i * (NCH // 8) + q)
        srcprep(i)
        return c
    jax.lax.fori_loop(0, 8, loop_p, 0)
    xw = up_s[pl.ds(PADR - 128, 136), :]
    src_s[6, pl.ds(PADR - 128, 128), :] = xw[1:129] + xw[2:130] + xw[3:131] + xw[4:132]

    row_head = jax.lax.broadcasted_iota(jnp.int32, (128, TQ), 0) // HP

    def scores(it, st_ref, m_ref):
        h = it // NQ
        qb = it % NQ
        q0 = pl.multiple_of(qb * TQ, TQ)
        g0 = pl.multiple_of((h // 4) * 128, 128)
        qt = qt_s[pl.ds(g0, 128), pl.ds(q0, TQ)]
        qt = jnp.where(row_head == h % 4, qt, jnp.zeros_like(qt))
        st = jnp.dot(k_s[h // 4], qt, preferred_element_type=F32)
        st_ref[...] = st
        m_ref[...] = jnp.max(st, axis=0, keepdims=True)

    def finish(it, st_ref, m_ref):
        h = it // NQ
        qb = it % NQ
        q0 = pl.multiple_of(qb * TQ, TQ)
        p = jnp.exp2(st_ref[...] - m_ref[...]).astype(BF16)
        h0 = pl.multiple_of(h * HP, HP)
        ot = jnp.dot(vt_s[pl.ds(h0, HP), :], p, preferred_element_type=F32)
        ot_s[pl.ds(h0, HP), pl.ds(q0, TQ)] = (ot / ot[DH:DH + 1, :]).astype(BF16)

    def attn_pair(i):
        it = 2 * i
        scores(it + 1, stb, mb)
        finish(it, sta, ma)
        scores(jnp.minimum(it + 2, 2 * NIT - 1), sta, ma)
        finish(it + 1, stb, mb)

    def kslice(sl):
        base = (sl // NCH) * 128
        zs = (par_s[sl, 0], par_s[sl, 1])
        w = (par_s[sl, 2], par_s[sl, 3])
        c1 = zs[0] + zs[0]
        c2 = zs[0] * zs[0] + zs[1] * zs[1]
        r0 = w[0]
        r1 = r0 * zs[0] - w[1] * zs[1]
        for b in range(128):
            if b >= 2:
                r0, r1 = r1, c1 * r1 - c2 * r0
            t = r0 if b == 0 else r1
            r = pl.multiple_of((base + b) * 8, 8)
            kac2_s[pl.ds(r, 8), :] += t[0:8] + t[8:16]

    def kslices(s0, n):
        for q in range(n):
            kslice(s0 + q)

    def kcopy(lo, hi):
        def body(j, c):
            r = pl.multiple_of((lo + 8 * j) * 8, 64)
            v = kac2_s[pl.ds(r, 64), :]
            for lb in range(4):
                kacc_s[lb, pl.ds(r, 64), :] = v[:, 128 * lb: 128 * (lb + 1)]
            return c
        jax.lax.fori_loop(0, (hi - lo) // 8, body, 0)

    def conv_d(d):
        r0 = kt_s[pl.ds(d, 1), :].astype(BF16).astype(F32)
        b0 = jax.lax.bitcast_convert_type(r0, U32)
        b1 = jax.lax.bitcast_convert_type(pltpu.roll(r0, 1, 1), U32)
        word = (b0 >> 16) | b1
        t32 = pltpu.roll(jnp.broadcast_to(word, (64, WID)), 0, 1, stride=2, stride_axis=0)
        w = pltpu.bitcast(t32, BF16)
        up = jnp.concatenate([jnp.zeros((16, 128), F32), ut_ref[d].astype(F32)], axis=0)
        acc = None
        for m in range(NT):
            t = jnp.dot(up[16 - m: 32 - m].astype(BF16), w[:, 128 * m: 128 * (m + 1)],
                        preferred_element_type=F32)
            acc = t if acc is None else acc + t
        yt_s[d] = acc

    def unit(ui, seg):
        ra = pl.multiple_of(tab_ref[ui, 0], 8)
        k0 = tab_ref[ui, 1]
        t0 = pl.multiple_of(tab_ref[ui, 2], BR)
        for hf in range(2):
            ls = pl.ds(256 * hf, 256)

            def kb(idx):
                r = pl.multiple_of(idx * 8, 8)
                return jnp.concatenate([kacc_s[2 * hf + lb, pl.ds(r, 8), :] for lb in range(2)], axis=1)[None]
            acc = y_s[pl.ds(t0, BR), ls].reshape(BR // 8, 8, 256)
            if seg == 2:
                plan = [(0, 0, 8, 0, 8), (1, 0, 8, 1, 8)]
            else:
                plan = [(2, 0, 16, 0, 4), (2, 64, 16, 8, 4), (3, 8, 16, 1, 4), (3, 72, 16, 9, 4)]
            for src, off, step, kof, cnt in plan:
                span = step * (cnt - 1)
                blk = src_s[src, pl.ds(ra - off - span, BR + span), ls]
                for e in range(cnt):
                    o = span - step * e
                    acc = acc + blk[o: o + BR].reshape(BR // 8, 8, 256) * kb(k0 + kof + 2 * e)
            y_s[pl.ds(t0, BR), ls] = acc.reshape(BR, 256)

    def kreduce(lo, hi):
        def body(j, c):
            r = pl.multiple_of((lo + 8 * j) * 8, 64)
            for lb in range(4):
                t = kacc_s[lb, pl.ds(r, 8, stride=8), :]
                for s in range(1, 8):
                    t = t + kacc_s[lb, pl.ds(r + s, 8, stride=8), :]
                kd_s[pl.ds(pl.multiple_of(lo + 8 * j, 8), 8), pl.ds(128 * lb, 128)] = t
            return c
        jax.lax.fori_loop(0, (hi - lo) // 8, body, 0)

    scores(0, sta, ma)

    def loop_a(i, c):
        attn_pair(i)
        kslices(SPI * i, SPI)
        return c
    jax.lax.fori_loop(0, IT_A, loop_a, 0)

    kcopy(0, 384)
    kreduce(0, 384)
    sub = jax.lax.broadcasted_iota(jnp.int32, (8, DP), 0)
    for blk in range(4):
        if blk < 2:
            rows = kd_s[pl.ds(128 * blk, 128), :]
        else:
            parts = []
            for b8 in range(16):
                acc = None
                for r in range(8):
                    l = 128 * blk + 8 * b8 + r
                    if l == 511:
                        v = jnp.zeros((8, DP), F32)
                    else:
                        v = jnp.broadcast_to(kd_s[pl.ds(_LIDX[_RL[l]], 1), :], (8, DP))
                    acc = v if acc is None else jnp.where(sub == r, v, acc)
                parts.append(acc)
            rows = jnp.concatenate(parts, axis=0)
        kt_s[:, pl.ds(128 * blk, 128)] = rows.T
    kt_s[:, pl.ds(512, 128)] = jnp.zeros((DP, 128), F32)

    def loop_b(j, c):
        attn_pair(IT_A + j)
        kslices(SPI * (IT_A + j), SPI)
        for q in range(DPB):
            conv_d(LOFF + j * DPB + q)
        return c
    jax.lax.fori_loop(0, IT_B, loop_b, 0)

    kcopy(384, 640)
    kreduce(384, 640)
    t = kacc_get(NLAG - 1)
    kd_s[pl.ds(640, 8), :] = jnp.broadcast_to(jnp.sum(t, axis=0, keepdims=True), (8, DP))

    def kbro(i, c):
        kacc_set(384 + i, jnp.broadcast_to(kd_s[pl.ds(384 + i, 1), :], (8, DP)))
        return c
    jax.lax.fori_loop(0, 257, kbro, 0)

    def loop_c(j, c):
        attn_pair(IT_A + IT_B + j)
        for q in range(U2PC):
            unit(j * U2PC + q, 2)
        for q in range(U3PC):
            unit(NU2 + j * U3PC + q, 3)
        for q in range(DPC):
            conv_d(jnp.minimum(LOFF + IT_B * DPB + j * DPC + q, DP - 1))
        return c
    jax.lax.fori_loop(0, IT_C, loop_c, 0)

    dsk = dsk_ref[...].astype(F32)
    lane = jax.lax.broadcasted_iota(jnp.int32, (128, 128), 1)
    k512 = kacc_get(384)[None]
    k1024 = kacc_get(512)[None]
    k2048 = kacc_get(640)[None]

    def fin(tb, c):
        r0 = pl.multiple_of(tb * 128, 128)
        y = y_s[pl.ds(r0, 128), :]
        for s, lag, kk in ((4, 512, k512), (5, 1024, k1024), (6, 2048, k2048)):
            a = jnp.maximum(PADR + r0 - lag, PADR - 128)
            e = src_s[s, pl.ds(pl.multiple_of(a, 8), 128), :]
            valid = (PADR + r0 - lag) >= PADR - 128
            e = jnp.where(valid, e, 0.0)
            y = y + (e.reshape(16, 8, DP) * kk).reshape(128, DP)
        yt = jnp.concatenate([yt_s[pl.ds(128 * db, 128), tb, :].T for db in range(4)], axis=1)
        y = y + yt
        ud = (u_ref[pl.ds(r0, 128), :].astype(F32) * dsk).astype(BF16).astype(F32)
        y = (y.astype(BF16).astype(F32) + ud).astype(BF16)
        a = jax.lax.dot_general(ot_s[:, pl.ds(r0, 128)], wo_ref[...], (((0,), (0,)), ((), ())),
                                preferred_element_type=F32).astype(BF16)
        o_ref[pl.ds(r0, 128), 0:384] = a[:, 0:384]
        o_ref[pl.ds(r0, 128), 384:512] = jnp.where(lane < LOFF, a[:, 384:512], y[:, 0:128])
        o_ref[pl.ds(r0, 128), 512:896] = y[:, 128:512]
        return c
    jax.lax.fori_loop(0, S // 128, fin, 0)


@jax.jit
def pallas_concat_heads__mha_block__ssm_conv_s4__prompt_kernel(
    A_x: jax.Array,
    A_wqkv: jax.Array,
    A_wo: jax.Array,
    B_u: jax.Array,
    B_A_re: jax.Array,
    B_A_im: jax.Array,
    B_B_re: jax.Array,
    B_B_im: jax.Array,
    B_C_re: jax.Array,
    B_C_im: jax.Array,
    B_log_dt: jax.Array,
    B_Dskip: jax.Array,
):
    x = A_x.reshape(S, D)
    w = jnp.pad(A_wqkv.reshape(D, 3, H, DH), ((0, 0), (0, 0), (0, 0), (0, HP - DH)))
    wq_t = w[:, 0].reshape(D, DP).T
    wk = w[:, 1].reshape(D, DP)
    wv_t = w[:, 2].reshape(D, DP).T
    wo = jnp.pad(A_wo.reshape(H, DH, D), ((0, 0), (0, HP - DH), (0, DP - D))).reshape(DP, DP)
    u = jnp.pad(B_u.reshape(S, D), ((0, 0), (LOFF, 0)))
    ut = u.T.reshape(DP, 16, 128)

    prm = jnp.stack([B_A_re, B_A_im, B_B_re, B_B_im, B_C_re, B_C_im])
    prm = jnp.pad(prm.transpose(0, 2, 1), ((0, 0), (0, 0), (LOFF, 0)))
    ldt = jnp.pad(B_log_dt.reshape(1, D), ((0, 0), (LOFF, 0)))
    dsk = jnp.pad(B_Dskip.reshape(1, D), ((0, 0), (LOFF, 0)))

    vmem = pl.BlockSpec(memory_space=pltpu.VMEM)
    out = pl.pallas_call(
        _kernel,
        out_shape=jax.ShapeDtypeStruct((S, 2 * D), BF16),
        in_specs=[pl.BlockSpec(memory_space=pltpu.SMEM)] + [vmem] * 10,
        out_specs=vmem,
        scratch_shapes=[
            pltpu.VMEM((DP, S), BF16),
            pltpu.VMEM((4, S, 128), BF16),
            pltpu.VMEM((DP, S), BF16),
            pltpu.VMEM((DP, S), BF16),
            pltpu.VMEM((S, TQ), F32),
            pltpu.VMEM((S, TQ), F32),
            pltpu.VMEM((1, TQ), F32),
            pltpu.VMEM((1, TQ), F32),
            pltpu.VMEM((5 * NCH, 4, NC, DP), F32),
            pltpu.VMEM((4, (NLAG + 7) * 8, 128), F32),
            pltpu.VMEM((640 * 8, DP), F32),
            pltpu.VMEM((NLAG + 7, DP), F32),
            pltpu.VMEM((DP, WID), F32),
            pltpu.VMEM((S + PADR + 8, DP), F32),
            pltpu.VMEM((NSRC, S + PADR, DP), F32),
            pltpu.VMEM((DP, 16, 128), F32),
            pltpu.VMEM((S, DP), F32),
        ],
        compiler_params=pltpu.CompilerParams(vmem_limit_bytes=120 * 1024 * 1024),
    )(jnp.asarray(_UNITS), x, wq_t, wk, wv_t, wo, u, ut, prm, ldt, dsk)
    return out.reshape(1, S, 2 * D)
```
